```python
import os as _os
_os.environ.setdefault("JAX_PLATFORMS", "cpu")
import jax
import jax.numpy as jnp

def _softmax(x, axis=-1):
    return jax.nn.softmax(x, axis=axis)
def _gelu(x):
    return jax.nn.gelu(x, approximate=True)
def _silu(x):
    return jax.nn.silu(x)
def _sigmoid(x):
    return jax.nn.sigmoid(x)
def _layernorm(x, axis=-1, eps=1e-5):
    m = jnp.mean(x, axis=axis, keepdims=True)
    v = jnp.var(x, axis=axis, keepdims=True)
    return (x - m) / jnp.sqrt(v + eps)
def _scatter_add(tgt, idx, src, axis=0):
    return tgt.at[idx].add(src)
def _segment_sum(src, seg, n):
    return jax.ops.segment_sum(src, seg, n)
class _Rng:
    def __init__(self, key):
        self._k = key
    def _next(self):
        self._k, sub = jax.random.split(self._k)
        return sub
    def normal(self, shape):
        return jax.random.normal(self._next(), shape, dtype=jnp.bfloat16)
    def randint(self, lo, hi, shape):
        return jax.random.randint(self._next(), shape, lo, hi, dtype=jnp.int32)
    def uniform(self, shape, lo=0.0, hi=1.0):
        return jax.random.uniform(self._next(), shape, jnp.bfloat16, lo, hi)
    def permutation(self, n):
        return jax.random.permutation(self._next(), n)


kernel_name = 'standalone__layernorm_linear__sampling'

def setup_inputs():
    _rng = _Rng(jax.random.key(int.from_bytes(__import__("os").urandom(4), "little")))
    _w = (lambda a: (lambda t: t.astype(jnp.bfloat16) if jnp.issubdtype(t.dtype, jnp.floating) else t)(jnp.asarray(a)))
    B, S, D = 1024, 32, 576
    return {
        "x": _w((lambda *s: _rng.normal(s) * 0.05)(B, S, D)),
        "g": _w((lambda *s: _rng.normal(s) * 0.05)(D) + 1.0),
        "b": _w((lambda *s: _rng.normal(s) * 0.05)(D)),
        "w": _w((lambda *s: _rng.normal(s) * 0.05)(D, D)),
    }

def reference(x, g, b, w):
    return (_layernorm(x, axis=-1) * g + b) @ w
```

```python
import functools

import jax
import jax.numpy as jnp
from jax import lax
from jax.experimental import pallas as pl
from jax.experimental.pallas import tpu as pltpu

EPS = 1e-5
KB = 64
LANES = 128
PAIR = 2 * LANES
ROWS = 96

TILES = ("cP", "dP", "eP", "aP1", "cQ", "dQ", "eQ", "bQ1",
         "R", "T", "aP2", "bQ2", "aU", "aV", "bU", "bV")
TILE = {name: i for i, name in enumerate(TILES)}

GROUPS = (
    (0, 1, 1.0, (("R", 0), ("bU", 0), ("cQ", 0), ("cP", 0), ("aU", 0), ("bQ1", 0), ("aP1", 0))),
    (2, 3, 0.5, (("R", 1), ("bV", 1), ("dQ", 1), ("dP", 1), ("aV", 1), ("bQ1", 1), ("aP1", 1))),
    (4, 5, 0.5, (("T", 0), ("bV", 0), ("cQ", 1), ("cP", 1), ("aV", 0), ("bQ2", 0), ("aP2", 0))),
    (6, 7, 1.0, (("T", 1), ("bU", 1), ("eQ", 1), ("eP", 1), ("aU", 1), ("bQ2", 1), ("aP2", 1))),
)

WEIGHT_TERMS = {
    ("R", 0): ((1, 0, 0), (1, 1, 1)), ("R", 1): ((1, 1, 3), (2, 0, 2)),
    ("T", 0): ((1, 0, 4), (1, 1, 5)), ("T", 1): ((1, 1, 7), (0.5, 0, 6)),
    ("aU", 0): ((1, 0, 0), (1, 0, 1)), ("aU", 1): ((1, 0, 6), (1, 0, 7)),
    ("bU", 0): ((1, 1, 0), (1, 1, 1)), ("bU", 1): ((1, 1, 6), (1, 1, 7)),
    ("aV", 0): ((1, 0, 4), (1, 0, 5)), ("aV", 1): ((1, 0, 2), (1, 0, 3)),
    ("bV", 0): ((1, 1, 4), (1, 1, 5)), ("bV", 1): ((1, 1, 2), (1, 1, 3)),
    ("cP", 0): ((-1, 1, 1),), ("cP", 1): ((-2, 1, 5),),
    ("cQ", 0): ((1, 0, 0),), ("cQ", 1): ((1, 0, 4),),
    ("dP", 0): ((-1 / 3, 0, 8), (2 / 3, 1, 8)), ("dP", 1): ((-1, 1, 3),),
    ("dQ", 0): ((-1 / 3, 0, 8), (2 / 3, 1, 8)), ("dQ", 1): ((1, 0, 2),),
    ("eP", 0): ((2 / 3, 0, 8), (-1 / 3, 1, 8)), ("eP", 1): ((-1, 1, 7),),
    ("eQ", 0): ((2 / 3, 0, 8), (-1 / 3, 1, 8)), ("eQ", 1): ((0.5, 0, 6),),
    ("aP1", 0): ((1, 0, 1), (-1, 1, 1)), ("aP1", 1): ((2, 0, 3), (-1, 1, 3)),
    ("aP2", 0): ((2, 0, 5), (-2, 1, 5)), ("aP2", 1): ((1, 0, 7), (-2, 1, 7)),
    ("bQ1", 0): ((1, 0, 0), (-1, 1, 0)), ("bQ1", 1): ((2, 0, 2), (-1, 1, 2)),
    ("bQ2", 0): ((1, 0, 4), (-1, 1, 4)), ("bQ2", 1): ((0.5, 0, 6), (-1, 1, 6)),
}
PANELS = ((0, 2), (1, 3), (4, 6), (5, 7), (8, 4), (8, 5))

PLAN = ((2, 4), (8, 1), (16, 7))
FINE_STEPS = 8
WRITE_START = 63
WRITE_SLICES = 4

f32, bf16, u32 = jnp.float32, jnp.bfloat16, jnp.uint32


def _tree_sum(parts):
    while len(parts) > 1:
        parts = [parts[i] + parts[i + 1] if i + 1 < len(parts) else parts[i]
                 for i in range(0, len(parts), 2)]
    return parts[0]


def _row_sum(a):
    return _tree_sum([a[i:i + 8] for i in range(0, a.shape[0], 8)])


def _rows(v, n):
    return jnp.concatenate([v] * (n // 8), axis=0)


def _segments(r0, n):
    out = []
    while n:
        m = min(n, KB - r0 % KB)
        out.append((r0 // KB, r0 % KB, m))
        r0, n = r0 + m, n - m
    return out


def _kernel(x_hbm, g_hbm, b_hbm, w_hbm, o_hbm,
            xbuf, obuf, wbuf, gbuf, bbuf, panels, lhs, bias, stage, slots,
            fine_sem, in_sem, out_sem, par_sem):
    D = wbuf.shape[0]
    half = D // 2
    nkb = D // KB
    S = xbuf.shape[0] // nkb
    per_slice = xbuf.shape[2] // PAIR
    steps = S * per_slice
    assert (nkb, per_slice) == (9, 4) and sum(u * n for u, n in PLAN) == steps
    fine_slices = FINE_STEPS // per_slice
    chunks = half // ROWS

    per_step = 16 // WRITE_SLICES
    batches = 0
    while (WRITE_START + batches * 32 // per_step
           >= per_slice * WRITE_SLICES * (batches + 1) - 1):
        batches += 1
    tail_start = WRITE_START + batches * 32 // per_step
    tail, nxt = {}, batches * WRITE_SLICES * per_slice
    for q in range(tail_start, steps):
        n = steps - nxt if q == steps - 1 else min(2, q + 1 - nxt)
        tail[q] = [t for t in range(nxt, nxt + n) if t != steps - 1]
        nxt += n
    assert tail_start >= steps - PLAN[-1][0]

    def read_fine(i):
        idx = (pl.ds((i >> 1) * nkb, nkb), slice(None),
               pl.ds(pl.multiple_of((i & 1) * (2 * PAIR), 2 * PAIR), 2 * PAIR))
        return pltpu.make_async_copy(x_hbm.at[idx], xbuf.at[idx], fine_sem.at[i])

    def read_slice(s):
        idx = pl.ds(s * nkb, nkb)
        return pltpu.make_async_copy(x_hbm.at[idx], xbuf.at[idx], in_sem.at[s])

    def write(idx, priority):
        pltpu.make_async_copy(obuf.at[idx], o_hbm.at[idx], out_sem).start(priority=priority)

    def write_part(g0, r0, c):
        write((pl.ds(g0, WRITE_SLICES * nkb), pl.ds(pl.multiple_of(r0, 8), 8),
               pl.ds(PAIR * c, PAIR)), c % 2)

    def write_steps(qs):
        for q in qs:
            for c in range(2):
                write((pl.ds(q // per_slice * nkb, nkb), slice(None),
                       pl.ds(q % per_slice * PAIR + c * LANES, LANES)), c)

    def write_last_rows(r0):
        for base in (r0, half + r0):
            for j, (kb, o, m) in enumerate(_segments(base, ROWS)):
                write(((S - 1) * nkb + kb, pl.ds(o, m),
                       pl.ds((per_slice - 1) * PAIR, PAIR)), j % 2)

    get_g = pltpu.make_async_copy(g_hbm, gbuf, par_sem.at[0])
    get_b = pltpu.make_async_copy(b_hbm, bbuf, par_sem.at[1])
    get_w = [pltpu.make_async_copy(w_hbm.at[pl.ds(o, n)], wbuf.at[pl.ds(o, n)], par_sem.at[2 + j])
             for j, (o, n) in enumerate(((0, 4 * KB), (4 * KB, 5 * KB)))]
    for copy in (get_g, get_b, *get_w):
        copy.start()
    for i in range(4):
        slots[i] = i % 2
    get_g.wait()
    get_b.wait()
    for i in range(FINE_STEPS // 2):
        read_fine(jnp.int32(i)).start()
    for s in range(fine_slices, S):
        read_slice(s).start()

    for copy, js in zip(get_w, ((0, 1), (2, 3, 4, 5))):
        copy.wait()
        for j in js:
            panels[j] = jnp.concatenate(
                [wbuf[k * KB:(k + 1) * KB, :] for k in PANELS[j]], axis=0).T

    def per_panel(ref):
        v = ref[...].astype(f32).reshape(1, D)
        return [jnp.concatenate([v[:, k * KB:(k + 1) * KB] for k in ks], axis=1) for ks in PANELS]

    left = lax.broadcasted_iota(jnp.int32, (1, LANES), 1) < KB
    b_lanes = per_panel(bbuf)[:5]
    b_lanes[4] = jnp.where(left, b_lanes[4], 0.0)
    bias[...] = _tree_sum([
        lax.dot_general(panels[j], jnp.broadcast_to(v, (LANES, LANES)).astype(bf16),
                        (((1,), (1,)), ((), ())), preferred_element_type=f32)
        for j, v in enumerate(b_lanes)])
    g_lanes = per_panel(gbuf)
    for r0 in range(0, half, 16):
        gw = {(h, j): panels[j, h * half + r0:h * half + r0 + 16, :].astype(f32) * g_lanes[j]
              for h in range(2) for j in range(len(PANELS))}
        for name in TILES:
            sides = []
            for side in range(2):
                acc = None
                for coef, h, k in WEIGHT_TERMS[name, side]:
                    v = gw[h, [ks[side] for ks in PANELS].index(k)]
                    if acc is None:
                        acc = v if coef == 1 else v * coef
                    else:
                        acc = acc + v if coef == 1 else acc - v if coef == -1 else acc + v * coef
                sides.append(acc)
            lhs[TILE[name], r0:r0 + 16, :] = jnp.where(left, *sides).astype(bf16)

    def load_x(at, kb, o, n):
        return xbuf[at[0] + kb, o:o + n, pl.ds(at[1], PAIR)].astype(f32)

    def pivot(at):
        return jnp.broadcast_to(load_x(at, 0, 0, 8)[0:1], (8, PAIR))

    def moments(at, kb, c):
        d = load_x(at, kb, 0, KB) - _rows(c, KB)
        return _row_sum(d), _row_sum(d * d)

    def mean_rstd(c, parts):
        m1, m2 = (jnp.broadcast_to(jnp.sum(_tree_sum(list(p)) * (1.0 / D), axis=0, keepdims=True),
                                   (8, PAIR)) for p in zip(*parts))
        return c + m1, lax.rsqrt(m2 - m1 * m1 + EPS)

    def normalize(at, piece, mean, rstd, slot):
        if piece < 16:
            ku, kv, scale, dests = GROUPS[piece // 4]
            o = 16 * (piece % 4)
            u, v = load_x(at, ku, o, 16), load_x(at, kv, o, 16)
            r0 = _rows(rstd[:, :LANES] if scale == 1 else rstd[:, :LANES] * scale, 16)
            r1 = _rows(rstd[:, LANES:], 16)
            u0 = (u[:, :LANES] - _rows(mean[:, :LANES], 16)) * r0
            v1 = (v[:, LANES:] - _rows(mean[:, LANES:], 16)) * r1
            d0 = (u[:, :LANES] - v[:, :LANES]) * r0
            d1 = (u[:, LANES:] - v[:, LANES:]) * r1
            e = u0 - v1
            for (name, side), val in zip(dests, (e, u0, d1, d0, v1, e - d1, e - d0)):
                stage[slot, TILE[name], side * KB + o:side * KB + o + 16, :] = val.astype(bf16)
        else:
            for o in (32 * (piece - 16), 32 * (piece - 16) + 16):
                xn = (load_x(at, 8, o, 16) - _rows(mean, 16)) * _rows(rstd, 16)
                for j, names in enumerate((("dP", "eP"), ("dQ", "eQ"))):
                    val = xn[:, j * LANES:(j + 1) * LANES].astype(bf16)
                    for name in names:
                        stage[slot, TILE[name], o:o + 16, :] = val

    def matmul(at, r0, slot, between):
        def products(*names):
            out = [jnp.dot(
                pltpu.bitcast(lhs.bitcast(u32)[TILE[n], r0 // 2:(r0 + ROWS) // 2, :], bf16),
                pltpu.bitcast(stage.bitcast(u32)[slot, TILE[n]], bf16),
                preferred_element_type=f32) for n in names]
            between()
            return out

        cP, dP, eP, aP = products("cP", "dP", "eP", "aP1")
        t = cP + dP + eP
        y00, y10 = t + eP + aP, t + dP
        cQ, dQ, eQ, bQ = products("cQ", "dQ", "eQ", "bQ1")
        t = cQ + dQ + eQ
        y01, y11 = t + eQ, t + dQ + bQ
        R, T, aP, bQ = products("R", "T", "aP2", "bQ2")
        t = R + T
        y00, y11 = y00 + t + T + aP, y11 - t + bQ
        aU, aV, bU, bV = products("aU", "aV", "bU", "bV")
        ta = aU + aV + bias[r0:r0 + ROWS, :]
        tb = bU + bV + bias[half + r0:half + r0 + ROWS, :]
        for base, ys in ((r0, (y00 + ta + aV, y01 + ta)), (half + r0, (y10 + tb + bV, y11 + tb))):
            y = jnp.concatenate(ys, axis=1).astype(bf16)
            p = 0
            for kb, o, m in _segments(base, ROWS):
                obuf[at[0] + kb, o:o + m, pl.ds(at[1], PAIR)] = y[p:p + m]
                p += m

    stage_f32 = stage.bitcast(f32)

    def parked(slot, i, j):
        return (slot, len(TILES) + i // 4, pl.ds(16 * (i % 4) + 8 * j, 8), slice(None))

    def block(q0, n, lo, hi, carry):
        if lo + 2 < FINE_STEPS:
            lax.fori_loop(jnp.minimum(q0 + 2, FINE_STEPS) >> 1,
                          jnp.minimum(q0 + n + 2, FINE_STEPS) >> 1,
                          lambda i, _: read_fine(i).wait(), None)
        if hi + n + 1 >= FINE_STEPS:
            lax.fori_loop(jnp.maximum(((q0 + 1) >> 2) + 1, fine_slices),
                          jnp.minimum(((q0 + n + 1) >> 2) + 1, S),
                          lambda s, _: read_slice(s).wait(), None)
        ld, st = (slots[0], slots[1]), (slots[2], slots[3])

        def at(j):
            if n % per_slice:
                return ((q0 + j) >> 2) * nkb, pl.multiple_of(((q0 + j) & 3) * PAIR, PAIR)
            s = (q0 >> 2) + j // per_slice
            return (jnp.minimum(s, S - 1) if j >= n else s) * nkb, j % per_slice * PAIR

        last = hi + n == steps
        gaps = 4 * chunks
        for p in range(n):
            c = pivot(at(p + 2))
            state = {"gap": 0, "next": None}

            def between():
                i = state["gap"]
                state["gap"] += 1
                for piece in range(18 * i // gaps, 18 * (i + 1) // gaps):
                    normalize(at(p + 1), piece, *carry, st[(p + 1) % 2])
                upto = min(nkb, nkb * (i + 1) // (gaps - 1))
                for kb in range(min(nkb, nkb * i // (gaps - 1)), upto):
                    for k, v in enumerate(moments(at(p + 2), kb, c)):
                        for j in range(2):
                            stage_f32[parked(st[0], 2 * kb + k, j)] = v[:, j * LANES:(j + 1) * LANES]
                if upto == nkb and state["next"] is None:
                    state["next"] = mean_rstd(c, [
                        [jnp.concatenate([stage_f32[parked(ld[0], 2 * kb + k, j)] for j in range(2)],
                                         axis=1) for k in range(2)] for kb in range(nkb)])

            for r0 in range(0, half, ROWS):
                matmul(at(p), r0, ld[p % 2], between)
                if last and p == n - 1:
                    pl.when(q0 == hi)(functools.partial(write_last_rows, r0))
            carry = state["next"]

            q = q0 + p
            if hi + p >= WRITE_START and lo + p < tail_start:
                due = jnp.logical_and(q >= WRITE_START, q < tail_start)
                d = (jnp.clip(q, WRITE_START, tail_start - 1) - WRITE_START) * (per_step // 4)
                for j in range(per_step):
                    pl.when(due)(functools.partial(
                        write_part, (d >> 3) * (WRITE_SLICES * nkb), ((d & 7) + j // 4) << 3, j % 4))
            if last and tail.get(hi + p):
                pl.when(q0 == hi)(functools.partial(write_steps, tail[hi + p]))
        return carry

    read_fine(jnp.int32(0)).wait()
    first = []
    for at in ((0, 0), (0, PAIR)):
        c = pivot(at)
        first.append(mean_rstd(c, [moments(at, kb, c) for kb in range(nkb)]))
    for piece in range(18):
        normalize((0, 0), piece, *first[0], 0)

    carry, lo = first[1], 0
    for n, count in PLAN:
        hi = lo + (count - 1) * n
        carry = lax.fori_loop(
            0, count, lambda i, c, n=n, lo=lo, hi=hi: block(lo + i * n, n, lo, hi, c), carry)
        lo = hi + n
    pltpu.make_async_copy(obuf, o_hbm, out_sem).wait()


@jax.jit
def pallas_standalone__layernorm_linear__sampling_kernel(
    x: jax.Array,
    g: jax.Array,
    b: jax.Array,
    w: jax.Array,
):
    B, S, D = x.shape
    view = (S * D // KB, KB, B)
    out = pl.pallas_call(
        _kernel,
        in_specs=[pl.BlockSpec(memory_space=pl.ANY)] * 4,
        out_specs=pl.BlockSpec(memory_space=pl.ANY),
        out_shape=jax.ShapeDtypeStruct(view, x.dtype),
        scratch_shapes=[
            pltpu.VMEM(view, bf16),
            pltpu.VMEM(view, bf16),
            pltpu.VMEM((D, D), bf16),
            pltpu.VMEM((D,), bf16),
            pltpu.VMEM((D,), bf16),
            pltpu.VMEM((len(PANELS), D, LANES), bf16),
            pltpu.VMEM((len(TILES), D // 2, LANES), bf16),
            pltpu.VMEM((D, LANES), f32),
            pltpu.VMEM((2, len(TILES) + 5, LANES, LANES), bf16),
            pltpu.SMEM((4,), jnp.int32),
            pltpu.SemaphoreType.DMA((FINE_STEPS // 2,)),
            pltpu.SemaphoreType.DMA((S,)),
            pltpu.SemaphoreType.DMA(()),
            pltpu.SemaphoreType.DMA((4,)),
        ],
        compiler_params=pltpu.CompilerParams(
            vmem_limit_bytes=100 * 1024 * 1024,
            disable_bounds_checks=True,
        ),
    )(jnp.transpose(x, (1, 2, 0)).reshape(view), g, b, w)
    return jnp.transpose(out.reshape(S, D, B), (2, 0, 1))
```

```python
import functools

import jax
import jax.numpy as jnp
from jax import lax
from jax.experimental import pallas as pl
from jax.experimental.pallas import tpu as pltpu

EPS = 1e-5
KB = 64
LANES = 128
PAIR = 2 * LANES
ROWS = 96

TILES = ("cP", "dP", "eP", "aP1", "cQ", "dQ", "eQ", "bQ1",
         "R", "T", "aP2", "bQ2", "aU", "aV", "bU", "bV")
TILE = {name: i for i, name in enumerate(TILES)}

GROUPS = (
    (0, 1, 1.0, (("R", 0), ("bU", 0), ("cQ", 0), ("cP", 0), ("aU", 0), ("bQ1", 0), ("aP1", 0))),
    (2, 3, 0.5, (("R", 1), ("bV", 1), ("dQ", 1), ("dP", 1), ("aV", 1), ("bQ1", 1), ("aP1", 1))),
    (4, 5, 0.5, (("T", 0), ("bV", 0), ("cQ", 1), ("cP", 1), ("aV", 0), ("bQ2", 0), ("aP2", 0))),
    (6, 7, 1.0, (("T", 1), ("bU", 1), ("eQ", 1), ("eP", 1), ("aU", 1), ("bQ2", 1), ("aP2", 1))),
)
PIECES = 18

PANELS = ((0, 2), (1, 3), (4, 6), (5, 7))

PLAN = ((2, 4), (8, 1), (16, 7))
FINE_READS = 6
WRITE_START = 60
WRITE_SLICES = 2

f32, bf16, u32 = jnp.float32, jnp.bfloat16, jnp.uint32


def _tree_sum(parts):
    while len(parts) > 1:
        parts = [parts[i] + parts[i + 1] if i + 1 < len(parts) else parts[i]
                 for i in range(0, len(parts), 2)]
    return parts[0]


def _row_sum(a):
    return _tree_sum([a[i:i + 8] for i in range(0, a.shape[0], 8)])


def _rows(v, n):
    return jnp.concatenate([v] * (n // 8), axis=0)


def _segments(r0, n):
    out = []
    while n:
        m = min(n, KB - r0 % KB)
        out.append((r0 // KB, r0 % KB, m))
        r0, n = r0 + m, n - m
    return out


def _kernel(x_hbm, g_hbm, b_hbm, w_hbm, o_hbm,
            xbuf, obuf, wbuf, gbuf, bbuf, panels, lhs, bias, stage, slots,
            fine_sem, in_sem, out_sem, par_sem):
    D = wbuf.shape[0]
    half = D // 2
    nkb = D // KB
    S = xbuf.shape[0] // nkb
    per_slice = xbuf.shape[2] // PAIR
    steps = S * per_slice
    assert (nkb, per_slice) == (9, 4) and sum(n * count for n, count in PLAN) == steps

    per_step = 16 // WRITE_SLICES
    batches = 0
    while (WRITE_START + batches * 32 // per_step
           >= per_slice * WRITE_SLICES * (batches + 1) - 1):
        batches += 1
    tail_start = WRITE_START + batches * 32 // per_step
    assert tail_start >= steps - PLAN[-1][0]

    def read_fine(i):
        idx = (pl.ds((i >> 1) * nkb, nkb), slice(None),
               pl.ds(pl.multiple_of((i & 1) * (2 * PAIR), 2 * PAIR), 2 * PAIR))
        return pltpu.make_async_copy(x_hbm.at[idx], xbuf.at[idx], fine_sem.at[i])

    def read_slices(s, n):
        idx = pl.ds(s * nkb, n * nkb)
        return pltpu.make_async_copy(x_hbm.at[idx], xbuf.at[idx], in_sem.at[s >> 1])

    def write(idx, priority):
        pltpu.make_async_copy(obuf.at[idx], o_hbm.at[idx], out_sem).start(priority=priority)

    def write_part(g0, r0, c):
        write((pl.ds(g0, WRITE_SLICES * nkb), pl.ds(pl.multiple_of(r0, 8), 8),
               pl.ds(PAIR * c, PAIR)), c % 2)

    def write_step(q):
        for c in range(2):
            write((pl.ds(q // per_slice * nkb, nkb), slice(None),
                   pl.ds(q % per_slice * PAIR + c * LANES, LANES)), c)

    def write_last_rows(r0):
        for j, (kb, o, m) in enumerate(_segments(r0, ROWS)):
            write(((S - 1) * nkb + kb, pl.ds(o, m), pl.ds((per_slice - 1) * PAIR, PAIR)), j % 2)

    get_g = pltpu.make_async_copy(g_hbm, gbuf, par_sem.at[0])
    get_b = pltpu.make_async_copy(b_hbm, bbuf, par_sem.at[1])
    get_w = [pltpu.make_async_copy(w_hbm.at[rows], wbuf.at[rows], par_sem.at[2 + j])
             for j, rows in enumerate((pl.ds(0, 4 * KB), pl.ds(4 * KB, 4 * KB), pl.ds(8 * KB, KB)))]
    for copy in (get_g, get_b, *get_w):
        copy.start()
    for i in range(4):
        slots[i] = i % 2
    get_g.wait()
    get_b.wait()
    for i in range(FINE_READS):
        read_fine(jnp.int32(i)).start()
    q0 = PLAN[0][0] * PLAN[0][1]
    assert FINE_READS // 2 == q0 // per_slice + 1
    for n, count in PLAN[1:]:
        for _ in range(count):
            s = q0 // per_slice + 1
            read_slices(s, min(n // per_slice, S - s)).start()
            q0 += n

    def lanes(ref, *blocks):
        v = ref[...].astype(f32).reshape(1, D)
        return jnp.concatenate([v[:, k * KB:(k + 1) * KB] for k in blocks], axis=1)

    def w_block(k):
        return wbuf[k * KB:(k + 1) * KB, :]

    left = lax.broadcasted_iota(jnp.int32, (1, LANES), 1) < KB

    def two(on_left, on_right):
        return jnp.where(left, on_left, on_right)

    bias_parts = []

    def add_panel(j, rows, b_lanes):
        rows = jnp.concatenate(rows, axis=0)
        panels.bitcast(u32)[j] = pltpu.bitcast(rows.T, u32)
        bias_parts.append(jnp.dot(jnp.broadcast_to(b_lanes, (16, LANES)).astype(bf16), rows,
                                  preferred_element_type=f32)[:8])

    for i in range(2):
        get_w[i].wait()
        for j in (2 * i, 2 * i + 1):
            add_panel(j, [w_block(k) for k in PANELS[j]], lanes(bbuf, *PANELS[j]))
    get_w[2].wait()
    top = lax.broadcasted_iota(jnp.int32, (KB, D), 1) < half
    add_panel(4, [w_block(8), jnp.where(top, w_block(4).astype(f32),
                                        w_block(5).astype(f32)).astype(bf16)],
              two(lanes(bbuf, 8, 8), 0.0))
    bias_row = _tree_sum(bias_parts)

    g_lanes = [[lanes(gbuf, *ks) for ks in (*PANELS, (8, 4 + h))] for h in range(2)]

    def weights(i, _):
        r0 = pl.multiple_of(i * 16, 16)
        a, b = ([panels[j, pl.ds(h * half + r0, 16), :].astype(f32) * g_lanes[h][j]
                 for j in range(5)] for h in range(2))
        a0, a2 = a[0] * two(1.0, 2.0), a[2] * two(1.0, 0.5)
        sa, sb = (a[0] + a[1], a[2] + a[3]), (b[0] + b[1], b[2] + b[3])
        third = (a[4] + b[4]) * (1 / 3)
        d8, e8 = b[4] - third, a[4] - third
        tiles = {
            "R": a0 + b[1], "T": a2 + b[3],
            "aU": two(sa[0], sa[1]), "aV": two(sa[1], sa[0]),
            "bU": two(sb[0], sb[1]), "bV": two(sb[1], sb[0]),
            "cP": two(b[1], b[4]) * two(-1.0, -2.0), "cQ": two(a[0], a[4]),
            "dP": two(d8, -b[1]), "dQ": two(d8, a[0]),
            "eP": two(e8, -b[3]), "eQ": two(e8, a2),
            "aP1": a[1] * two(1.0, 2.0) - b[1], "aP2": a[3] * two(2.0, 1.0) - (b[3] + b[3]),
            "bQ1": a0 - b[0], "bQ2": a2 - b[2],
        }
        for name in TILES:
            lhs[TILE[name], pl.ds(r0, 16), :] = tiles[name].astype(bf16)

    lax.fori_loop(0, half // 16, weights, None, unroll=6)

    def load_x(at, kb, o, n):
        return xbuf[at[0] + kb, o:o + n, pl.ds(at[1], PAIR)].astype(f32)

    def pivot(at):
        return jnp.broadcast_to(load_x(at, 0, 0, 8)[0:1], (8, PAIR))

    def moments(at, kb, c):
        d = load_x(at, kb, 0, KB) - _rows(c, KB)
        return _row_sum(d), _row_sum(d * d)

    def mean_rstd(c, parts):
        m1, m2 = (jnp.broadcast_to(jnp.sum(_tree_sum(list(p)) * (1.0 / D), axis=0, keepdims=True),
                                   (8, PAIR)) for p in zip(*parts))
        return c + m1, lax.rsqrt(m2 - m1 * m1 + EPS)

    def normalize(at, piece, mean, rstd, slot):
        if piece < 16:
            ku, kv, scale, dests = GROUPS[piece // 4]
            o = 16 * (piece % 4)
            u, v = load_x(at, ku, o, 16), load_x(at, kv, o, 16)
            r0 = _rows(rstd[:, :LANES] if scale == 1 else rstd[:, :LANES] * scale, 16)
            r1 = _rows(rstd[:, LANES:], 16)
            u0 = (u[:, :LANES] - _rows(mean[:, :LANES], 16)) * r0
            v1 = (v[:, LANES:] - _rows(mean[:, LANES:], 16)) * r1
            d0 = (u[:, :LANES] - v[:, :LANES]) * r0
            d1 = (u[:, LANES:] - v[:, LANES:]) * r1
            e = u0 - v1
            for (name, side), val in zip(dests, (e, u0, d1, d0, v1, e - d1, e - d0)):
                stage[slot, TILE[name], side * KB + o:side * KB + o + 16, :] = val.astype(bf16)
        else:
            for o in (32 * (piece - 16), 32 * (piece - 16) + 16):
                xn = (load_x(at, 8, o, 16) - _rows(mean, 16)) * _rows(rstd, 16)
                for j, names in enumerate((("dP", "eP"), ("dQ", "eQ"))):
                    val = xn[:, j * LANES:(j + 1) * LANES].astype(bf16)
                    for name in names:
                        stage[slot, TILE[name], o:o + 16, :] = val

    def matmul(at, r0, slot, between):
        def products(*names):
            out = [jnp.dot(
                pltpu.bitcast(lhs.bitcast(u32)[TILE[n], r0 // 2:(r0 + ROWS) // 2, :], bf16),
                pltpu.bitcast(stage.bitcast(u32)[slot, TILE[n]], bf16),
                preferred_element_type=f32) for n in names]
            between()
            return out

        cP, dP, eP, aP = products("cP", "dP", "eP", "aP1")
        t = cP + dP + eP
        y00, y10 = t + eP + aP, t + dP
        cQ, dQ, eQ, bQ = products("cQ", "dQ", "eQ", "bQ1")
        t = cQ + dQ + eQ
        y01, y11 = t + eQ, t + dQ + bQ
        R, T, aP, bQ = products("R", "T", "aP2", "bQ2")
        t = R + T
        y00, y11 = y00 + t + T + aP, y11 - t + bQ
        aU, aV, bU, bV = products("aU", "aV", "bU", "bV")
        ta = aU + aV + bias[r0:r0 + ROWS, :]
        tb = bU + bV + bias[half + r0:half + r0 + ROWS, :]
        for base, ys in ((r0, (y00 + ta + aV, y01 + ta)), (half + r0, (y10 + tb + bV, y11 + tb))):
            y = jnp.concatenate(ys, axis=1).astype(bf16)
            p = 0
            for kb, o, m in _segments(base, ROWS):
                obuf[at[0] + kb, o:o + m, pl.ds(at[1], PAIR)] = y[p:p + m]
                p += m

    stage_f32 = stage.bitcast(f32)

    def parked(slot, i, j):
        return (slot, len(TILES) + i // 4, pl.ds(16 * (i % 4) + 8 * j, 8), slice(None))

    def step(at, p, norm, ld, st, after_rows):
        c = pivot(at(p + 2))
        gaps = 4 * (half // ROWS)
        gap, out = iter(range(gaps)), []

        def between():
            i = next(gap)
            for piece in range(PIECES * i // gaps, PIECES * (i + 1) // gaps):
                normalize(at(p + 1), piece, *norm, st[(p + 1) % 2])
            if 1 <= i <= nkb:
                for k, v in enumerate(moments(at(p + 2), i - 1, c)):
                    for j in range(2):
                        stage_f32[parked(st[0], 2 * (i - 1) + k, j)] = v[:, j * LANES:(j + 1) * LANES]
            if i == nkb:
                out.extend(mean_rstd(c, [
                    [jnp.concatenate([stage_f32[parked(ld[0], 2 * kb + k, j)] for j in range(2)],
                                     axis=1) for k in range(2)] for kb in range(nkb)]))

        for r0 in range(0, half, ROWS):
            matmul(at(p), r0, ld[p % 2], between)
            after_rows(r0)
        return tuple(out)

    def wait_if(cond, copy):
        lax.fori_loop(0, jnp.where(cond, slots[1], 0), lambda i, _: copy().wait(), None)

    def block(q0, n, lo, hi, norm):
        last = hi + n == steps
        m = n // per_slice
        if not m:
            wait_if(True, lambda: read_fine((q0 >> 1) + 1))
        else:
            wait_if(q0 + n < steps, lambda: read_slices(jnp.minimum((q0 >> 2) + 1, S - m), m))
            if last:
                wait_if(q0 == hi, lambda: read_slices(jnp.minimum((q0 >> 2) + 1, S - m + 1), m - 1))
        ld, st = (slots[0], slots[1]), (slots[2], slots[3])

        def at(j):
            if not m:
                return ((q0 + j) >> 2) * nkb, pl.multiple_of(((q0 + j) & 3) * PAIR, PAIR)
            s = (q0 >> 2) + j // per_slice
            return (jnp.minimum(s, S - 1) if j >= n else s) * nkb, j % per_slice * PAIR

        for p in range(n):
            def after_rows(r0):
                if last and p == n - 1:
                    for base in (r0, half + r0):
                        pl.when(q0 == hi)(functools.partial(write_last_rows, base))

            norm = step(at, p, norm, ld, st, after_rows)
            q = q0 + p
            if hi + p >= WRITE_START and lo + p < tail_start:
                due = jnp.logical_and(q >= WRITE_START, q < tail_start)
                d = (jnp.clip(q, WRITE_START, tail_start - 1) - WRITE_START) * (per_step // 4)
                for j in range(per_step):
                    pl.when(due)(functools.partial(
                        write_part, (d >> 3) * (WRITE_SLICES * nkb), ((d & 7) + j // 4) << 3, j % 4))
            if last and hi + p >= tail_start:
                first = batches * WRITE_SLICES * per_slice if hi + p == tail_start else hi + p
                for t in range(first, min(hi + p + 1, steps - 1)):
                    pl.when(q0 == hi)(functools.partial(write_step, t))
        return norm

    def whole_norm(at):
        c = pivot(at)
        return mean_rstd(c, [moments(at, kb, c) for kb in range(nkb)])

    read_fine(jnp.int32(0)).wait()
    bias[...] = _rows(bias_row, LANES).T
    norm = whole_norm((0, 0))
    for piece in range(PIECES):
        normalize((0, 0), piece, *norm, 0)
    norm = whole_norm((0, PAIR))

    lo = 0
    for n, count in PLAN:
        hi = lo + (count - 1) * n
        norm = lax.fori_loop(
            0, count, lambda i, c, n=n, lo=lo, hi=hi: block(lo + i * n, n, lo, hi, c), norm)
        if not lo:
            lax.fori_loop(count + slots[1], FINE_READS, lambda i, _: read_fine(i).wait(), None)
        lo = hi + n
    pltpu.make_async_copy(obuf, o_hbm, out_sem).wait()


@jax.jit
def pallas_standalone__layernorm_linear__sampling_kernel(
    x: jax.Array,
    g: jax.Array,
    b: jax.Array,
    w: jax.Array,
):
    B, S, D = x.shape
    view = (S * D // KB, KB, B)
    out = pl.pallas_call(
        _kernel,
        in_specs=[pl.BlockSpec(memory_space=pl.ANY)] * 4,
        out_specs=pl.BlockSpec(memory_space=pl.ANY),
        out_shape=jax.ShapeDtypeStruct(view, x.dtype),
        scratch_shapes=[
            pltpu.VMEM(view, bf16),
            pltpu.VMEM(view, bf16),
            pltpu.VMEM((D, D), bf16),
            pltpu.VMEM((D,), bf16),
            pltpu.VMEM((D,), bf16),
            pltpu.VMEM((len(PANELS) + 1, D, LANES), bf16),
            pltpu.VMEM((len(TILES), D // 2, LANES), bf16),
            pltpu.VMEM((D, LANES), f32),
            pltpu.VMEM((2, len(TILES) + 5, LANES, LANES), bf16),
            pltpu.SMEM((4,), jnp.int32),
            pltpu.SemaphoreType.DMA((FINE_READS,)),
            pltpu.SemaphoreType.DMA((S // 2,)),
            pltpu.SemaphoreType.DMA(()),
            pltpu.SemaphoreType.DMA((5,)),
        ],
        compiler_params=pltpu.CompilerParams(
            vmem_limit_bytes=100 * 1024 * 1024,
            disable_bounds_checks=True,
            disable_semaphore_checks=True,
        ),
    )(jnp.transpose(x, (1, 2, 0)).reshape(view), g, b, w)
    return jnp.transpose(out.reshape(S, D, B), (2, 0, 1))
```

```python
import functools

import jax
import jax.numpy as jnp
from jax import lax
from jax.experimental import pallas as pl
from jax.experimental.pallas import tpu as pltpu

EPS = 1e-5
KB = 64
LANES = 128
PAIR = 2 * LANES
ROWS = 96

TILES = ("cP", "dP", "eP", "aP1", "cQ", "dQ", "eQ", "bQ1",
         "R", "T", "aP2", "bQ2", "aU", "aV", "bU", "bV")
TILE = {name: i for i, name in enumerate(TILES)}

GROUPS = (
    (0, 1, 1.0, (("R", 0), ("bU", 0), ("cQ", 0), ("cP", 0), ("aU", 0), ("bQ1", 0), ("aP1", 0))),
    (2, 3, 0.5, (("R", 1), ("bV", 1), ("dQ", 1), ("dP", 1), ("aV", 1), ("bQ1", 1), ("aP1", 1))),
    (4, 5, 0.5, (("T", 0), ("bV", 0), ("cQ", 1), ("cP", 1), ("aV", 0), ("bQ2", 0), ("aP2", 0))),
    (6, 7, 1.0, (("T", 1), ("bU", 1), ("eQ", 1), ("eP", 1), ("aU", 1), ("bQ2", 1), ("aP2", 1))),
)
PIECES = 18

PANELS = ((0, 2), (1, 3), (4, 6), (5, 7))

PLAN = ((4, 1), (8, 3), (24, 4))
WRITE_START = 60
WRITE_SLICES = 2

GAPS = 12


def _spread(tasks, first, last):
    return [(first + i * (last - first + 1) // len(tasks), t) for i, t in enumerate(tasks)]


TILES_ONLY = [(-(-GAPS * (i + 1) // PIECES) - 1, ("tiles", i)) for i in range(PIECES)]
STEADY = TILES_ONLY + [(k + 1, ("sums", 2, k)) for k in range(9)] + [(9, ("norm", 2))]
CATCH_UP = (_spread([("sums", 1, k) for k in range(9)], 0, 3) + [(3, ("norm", 1))]
            + _spread([("tiles", i) for i in range(PIECES)], 4, 11)
            + _spread([("sums", 2, k) for k in range(9)], 4, 10) + [(10, ("norm", 2))])

f32, bf16, u32 = jnp.float32, jnp.bfloat16, jnp.uint32


def _tree_sum(parts):
    while len(parts) > 1:
        parts = [parts[i] + parts[i + 1] if i + 1 < len(parts) else parts[i]
                 for i in range(0, len(parts), 2)]
    return parts[0]


def _row_sum(a):
    return _tree_sum([a[i:i + 8] for i in range(0, a.shape[0], 8)])


def _rows(v, n):
    return jnp.concatenate([v] * (n // 8), axis=0)


def _segments(r0, n):
    out = []
    while n:
        m = min(n, KB - r0 % KB)
        out.append((r0 // KB, r0 % KB, m))
        r0, n = r0 + m, n - m
    return out


def _kernel(x_hbm, g_hbm, b_hbm, w_hbm, o_hbm,
            xbuf, obuf, wbuf, panels, lhs, bias, stage, gbuf, bbuf, slots,
            step_sem, slice_sem, out_sem, par_sem):
    D = wbuf.shape[0]
    half = D // 2
    nkb = D // KB
    S = xbuf.shape[0] // nkb
    per_slice = xbuf.shape[2] // PAIR
    steps = S * per_slice
    assert (nkb, per_slice, 4 * half // ROWS) == (9, 4, GAPS)
    assert per_slice + sum(n * count for n, count in PLAN) == steps

    per_step = 16 // WRITE_SLICES
    batches = 0
    while (WRITE_START + batches * 32 // per_step
           >= per_slice * WRITE_SLICES * (batches + 1) - 1):
        batches += 1
    tail_start = WRITE_START + batches * 32 // per_step
    assert tail_start >= steps - PLAN[-1][0]

    def read_steps(q, n):
        idx = (pl.ds(q // per_slice * nkb, nkb), slice(None),
               pl.ds(q % per_slice * PAIR, n * PAIR))
        return pltpu.make_async_copy(x_hbm.at[idx], xbuf.at[idx], step_sem.at[q])

    def read_slices(s, n):
        idx = pl.ds(s * nkb, n * nkb)
        return pltpu.make_async_copy(x_hbm.at[idx], xbuf.at[idx], slice_sem.at[s])

    def write(idx, priority):
        pltpu.make_async_copy(obuf.at[idx], o_hbm.at[idx], out_sem).start(priority=priority)

    def write_part(g0, r0, c):
        write((pl.ds(g0, WRITE_SLICES * nkb), pl.ds(pl.multiple_of(r0, 8), 8),
               pl.ds(PAIR * c, PAIR)), c % 2)

    def write_step(q):
        for c in range(2):
            write((pl.ds(q // per_slice * nkb, nkb), slice(None),
                   pl.ds(q % per_slice * PAIR + c * LANES, LANES)), c)

    def write_last_rows(r0):
        for j, (kb, o, m) in enumerate(_segments(r0, ROWS)):
            write(((S - 1) * nkb + kb, pl.ds(o, m), pl.ds((per_slice - 1) * PAIR, PAIR)), j % 2)

    get_g = pltpu.make_async_copy(g_hbm, gbuf, par_sem.at[0])
    get_b = pltpu.make_async_copy(b_hbm, bbuf, par_sem.at[1])
    get_w = [pltpu.make_async_copy(w_hbm.at[rows], wbuf.at[rows], par_sem.at[2 + j])
             for j, rows in enumerate((pl.ds(0, 4 * KB), pl.ds(4 * KB, 5 * KB)))]
    for copy in (get_g, get_b, *get_w):
        copy.start()
    for i in range(4):
        slots[i] = i % 2
    get_g.wait()
    get_b.wait()
    for q, n in ((0, 2), (2, 1), (3, 1), (4, 2), (6, 2)):
        read_steps(q, n).start()
    q0 = per_slice
    for n, count in PLAN:
        for _ in range(count):
            s = q0 // per_slice + 1
            read_slices(s, min(n // per_slice, S - s)).start()
            q0 += n

    def lanes(ref, *blocks):
        v = ref[...].astype(f32).reshape(1, D)
        return jnp.concatenate([v[:, k * KB:(k + 1) * KB] for k in blocks], axis=1)

    def w_block(k):
        return wbuf[k * KB:(k + 1) * KB, :]

    left = lax.broadcasted_iota(jnp.int32, (1, LANES), 1) < KB

    def two(on_left, on_right):
        return jnp.where(left, on_left, on_right)

    bias_parts = []

    def add_panel(j, rows, b_lanes):
        rows = jnp.concatenate(rows, axis=0)
        panels.bitcast(u32)[j] = pltpu.bitcast(rows.T, u32)
        bias_parts.append(jnp.dot(jnp.broadcast_to(b_lanes, (16, LANES)).astype(bf16), rows,
                                  preferred_element_type=f32)[:8])

    for i in range(2):
        get_w[i].wait()
        for j in (2 * i, 2 * i + 1):
            add_panel(j, [w_block(k) for k in PANELS[j]], lanes(bbuf, *PANELS[j]))
    top = lax.broadcasted_iota(jnp.int32, (KB, D), 1) < half
    add_panel(4, [w_block(8), jnp.where(top, w_block(4).astype(f32),
                                        w_block(5).astype(f32)).astype(bf16)],
              two(lanes(bbuf, 8, 8), 0.0))
    bias_row = _tree_sum(bias_parts)

    g_lanes = [[lanes(gbuf, *ks) for ks in (*PANELS, (8, 4 + h))] for h in range(2)]

    def weights(i, _):
        r0 = pl.multiple_of(i * 16, 16)
        a, b = ([panels[j, pl.ds(h * half + r0, 16), :].astype(f32) * g_lanes[h][j]
                 for j in range(5)] for h in range(2))
        a0, a2 = a[0] * two(1.0, 2.0), a[2] * two(1.0, 0.5)
        sa, sb = (a[0] + a[1], a[2] + a[3]), (b[0] + b[1], b[2] + b[3])
        third = (a[4] + b[4]) * (1 / 3)
        d8, e8 = b[4] - third, a[4] - third
        tiles = {
            "R": a0 + b[1], "T": a2 + b[3],
            "aU": two(sa[0], sa[1]), "aV": two(sa[1], sa[0]),
            "bU": two(sb[0], sb[1]), "bV": two(sb[1], sb[0]),
            "cP": two(b[1], b[4]) * two(-1.0, -2.0), "cQ": two(a[0], a[4]),
            "dP": two(d8, -b[1]), "dQ": two(d8, a[0]),
            "eP": two(e8, -b[3]), "eQ": two(e8, a2),
            "aP1": a[1] * two(1.0, 2.0) - b[1], "aP2": a[3] * two(2.0, 1.0) - (b[3] + b[3]),
            "bQ1": a0 - b[0], "bQ2": a2 - b[2],
        }
        for name in TILES:
            lhs[TILE[name], pl.ds(r0, 16), :] = tiles[name].astype(bf16)

    lax.fori_loop(0, half // 16, weights, None, unroll=6)

    def load_x(at, kb, o, n):
        return xbuf[at[0] + kb, o:o + n, pl.ds(at[1], PAIR)].astype(f32)

    def pivot(at):
        return jnp.broadcast_to(load_x(at, 0, 0, 8)[0:1], (8, PAIR))

    def moments(at, kb, c):
        d = load_x(at, kb, 0, KB) - _rows(c, KB)
        return _row_sum(d), _row_sum(d * d)

    def mean_rstd(c, parts):
        m1, m2 = (jnp.broadcast_to(jnp.sum(_tree_sum(list(p)) * (1.0 / D), axis=0, keepdims=True),
                                   (8, PAIR)) for p in zip(*parts))
        return c + m1, lax.rsqrt(m2 - m1 * m1 + EPS)

    def normalize(at, piece, mean, rstd, slot):
        if piece < 16:
            ku, kv, scale, dests = GROUPS[piece // 4]
            o = 16 * (piece % 4)
            u, v = load_x(at, ku, o, 16), load_x(at, kv, o, 16)
            r0 = _rows(rstd[:, :LANES] if scale == 1 else rstd[:, :LANES] * scale, 16)
            r1 = _rows(rstd[:, LANES:], 16)
            u0 = (u[:, :LANES] - _rows(mean[:, :LANES], 16)) * r0
            v1 = (v[:, LANES:] - _rows(mean[:, LANES:], 16)) * r1
            d0 = (u[:, :LANES] - v[:, :LANES]) * r0
            d1 = (u[:, LANES:] - v[:, LANES:]) * r1
            e = u0 - v1
            for (name, side), val in zip(dests, (e, u0, d1, d0, v1, e - d1, e - d0)):
                stage[slot, TILE[name], side * KB + o:side * KB + o + 16, :] = val.astype(bf16)
        else:
            for o in (32 * (piece - 16), 32 * (piece - 16) + 16):
                xn = (load_x(at, 8, o, 16) - _rows(mean, 16)) * _rows(rstd, 16)
                for j, names in enumerate((("dP", "eP"), ("dQ", "eQ"))):
                    val = xn[:, j * LANES:(j + 1) * LANES].astype(bf16)
                    for name in names:
                        stage[slot, TILE[name], o:o + 16, :] = val

    def matmul(at, r0, slot, between):
        def products(*names):
            out = [jnp.dot(
                pltpu.bitcast(lhs.bitcast(u32)[TILE[n], r0 // 2:(r0 + ROWS) // 2, :], bf16),
                pltpu.bitcast(stage.bitcast(u32)[slot, TILE[n]], bf16),
                preferred_element_type=f32) for n in names]
            between()
            return out

        cP, dP, eP, aP = products("cP", "dP", "eP", "aP1")
        t = cP + dP + eP
        y00, y10 = t + eP + aP, t + dP
        cQ, dQ, eQ, bQ = products("cQ", "dQ", "eQ", "bQ1")
        t = cQ + dQ + eQ
        y01, y11 = t + eQ, t + dQ + bQ
        R, T, aP, bQ = products("R", "T", "aP2", "bQ2")
        t = R + T
        y00, y11 = y00 + t + T + aP, y11 - t + bQ
        aU, aV, bU, bV = products("aU", "aV", "bU", "bV")
        ta = aU + aV + bias[r0:r0 + ROWS, :]
        tb = bU + bV + bias[half + r0:half + r0 + ROWS, :]
        for base, ys in ((r0, (y00 + ta + aV, y01 + ta)), (half + r0, (y10 + tb + bV, y11 + tb))):
            y = jnp.concatenate(ys, axis=1).astype(bf16)
            p = 0
            for kb, o, m in _segments(base, ROWS):
                obuf[at[0] + kb, o:o + m, pl.ds(at[1], PAIR)] = y[p:p + m]
                p += m

    stage_f32 = stage.bitcast(f32)

    def parked(slot, i, j):
        return (slot, len(TILES) + i // 4, pl.ds(16 * (i % 4) + 8 * j, 8), slice(None))

    def step(at, p, norm, ld, st, tasks, after_rows=lambda r0: None):
        gap, norms, pivots = iter(range(GAPS)), {1: norm, 2: None}, {}

        def between():
            i = next(gap)
            for kind, *args in (task for g, task in tasks if g == i):
                if kind == "tiles":
                    normalize(at(p + 1), *args, *norms[1], st[(p + 1) % 2])
                    continue
                ahead = args[0]
                if ahead not in pivots:
                    pivots[ahead] = pivot(at(p + ahead))
                if kind == "sums":
                    for k, v in enumerate(moments(at(p + ahead), args[1], pivots[ahead])):
                        for j in range(2):
                            stage_f32[parked(st[0], 2 * args[1] + k, j)] = (
                                v[:, j * LANES:(j + 1) * LANES])
                else:
                    norms[ahead] = mean_rstd(pivots[ahead], [
                        [jnp.concatenate([stage_f32[parked(ld[0], 2 * kb + k, j)] for j in range(2)],
                                         axis=1) for k in range(2)] for kb in range(nkb)])

        for r0 in range(0, half, ROWS):
            matmul(at(p), r0, ld[p % 2], between)
            after_rows(r0)
        return norms[2]

    def stage_slots():
        return (slots[0], slots[1]), (slots[2], slots[3])

    def wait_if(cond, read, *ranges):
        def wait(i, _):
            for r in ranges:
                read(*r).wait()

        lax.fori_loop(0, jnp.where(cond, slots[1], 0), wait, None)

    def block(q0, n, lo, hi, norm):
        last = hi + n == steps
        m = n // per_slice
        wait_if(q0 + n < steps, read_slices, (jnp.minimum((q0 >> 2) + 1, S - m), m))
        if last:
            wait_if(q0 == hi, read_slices, (S - m + 1, m - 1))
        ld, st = stage_slots()

        def at(j):
            s = (q0 >> 2) + j // per_slice
            return (jnp.minimum(s, S - 1) if j >= n else s) * nkb, j % per_slice * PAIR

        for p in range(n):
            def after_rows(r0):
                if last and p == n - 1:
                    for base in (r0, half + r0):
                        pl.when(q0 == hi)(functools.partial(write_last_rows, base))

            norm = step(at, p, norm, ld, st, STEADY, after_rows)
            q = q0 + p
            if hi + p >= WRITE_START and lo + p < tail_start:
                due = jnp.logical_and(q >= WRITE_START, q < tail_start)
                d = (jnp.clip(q, WRITE_START, tail_start - 1) - WRITE_START) * (per_step // 4)
                for j in range(per_step):
                    pl.when(due)(functools.partial(
                        write_part, (d >> 3) * (WRITE_SLICES * nkb), ((d & 7) + j // 4) << 3, j % 4))
            if last and hi + p >= tail_start:
                first = batches * WRITE_SLICES * per_slice if hi + p == tail_start else hi + p
                for t in range(first, min(hi + p + 1, steps - 1)):
                    pl.when(q0 == hi)(functools.partial(write_step, t))
        return norm

    def first_at(q):
        return q // per_slice * nkb, q % per_slice * PAIR

    read_steps(0, 2).wait()
    c = pivot(first_at(0))
    norm = mean_rstd(c, [moments(first_at(0), kb, c) for kb in range(nkb)])
    for piece in range(PIECES):
        normalize(first_at(0), piece, *norm, 0)
    wait_if(True, read_steps, (2, 1))
    bias[...] = _rows(bias_row, LANES).T
    ld, st = stage_slots()
    step(first_at, 1, step(first_at, 0, None, ld, st, CATCH_UP), ld, st, TILES_ONLY)
    wait_if(True, read_steps, (3, 1), (4, 2))
    ld, st = stage_slots()
    norm = step(first_at, 3, step(first_at, 2, None, ld, st, CATCH_UP), ld, st, STEADY)
    wait_if(True, read_steps, (6, 2))

    lo = per_slice
    for n, count in PLAN:
        hi = lo + (count - 1) * n
        norm = lax.fori_loop(
            0, count, lambda i, c, n=n, lo=lo, hi=hi: block(lo + i * n, n, lo, hi, c), norm)
        lo = hi + n
    pltpu.make_async_copy(obuf, o_hbm, out_sem).wait()


@jax.jit
def pallas_standalone__layernorm_linear__sampling_kernel(
    x: jax.Array,
    g: jax.Array,
    b: jax.Array,
    w: jax.Array,
):
    B, S, D = x.shape
    view = (S * D // KB, KB, B)
    out = pl.pallas_call(
        _kernel,
        in_specs=[pl.BlockSpec(memory_space=pl.ANY)] * 4,
        out_specs=pl.BlockSpec(memory_space=pl.ANY),
        out_shape=jax.ShapeDtypeStruct(view, x.dtype),
        scratch_shapes=[
            pltpu.VMEM(view, bf16),
            pltpu.VMEM(view, bf16),
            pltpu.VMEM((D, D), bf16),
            pltpu.VMEM((len(PANELS) + 1, D, LANES), bf16),
            pltpu.VMEM((len(TILES), D // 2, LANES), bf16),
            pltpu.VMEM((D, LANES), f32),
            pltpu.VMEM((2, len(TILES) + 5, LANES, LANES), bf16),
            pltpu.VMEM((D,), bf16),
            pltpu.VMEM((D,), bf16),
            pltpu.SMEM((4,), jnp.int32),
            pltpu.SemaphoreType.DMA((8,)),
            pltpu.SemaphoreType.DMA((S,)),
            pltpu.SemaphoreType.DMA(()),
            pltpu.SemaphoreType.DMA((4,)),
        ],
        compiler_params=pltpu.CompilerParams(
            vmem_limit_bytes=100 * 1024 * 1024,
            disable_bounds_checks=True,
            disable_semaphore_checks=True,
        ),
    )(jnp.transpose(x, (1, 2, 0)).reshape(view), g, b, w)
    return jnp.transpose(out.reshape(S, D, B), (2, 0, 1))
```
